```python
import jax
import jax.numpy as jnp

def _softmax(x, axis=-1):
    return jax.nn.softmax(x, axis=axis)
def _gelu(x):
    return jax.nn.gelu(x, approximate=True)
def _silu(x):
    return jax.nn.silu(x)
def _sigmoid(x):
    return jax.nn.sigmoid(x)
def _layernorm(x, axis=-1, eps=1e-5):
    m = jnp.mean(x, axis=axis, keepdims=True)
    v = jnp.var(x, axis=axis, keepdims=True)
    return (x - m) / jnp.sqrt(v + eps)
def _scatter_add(tgt, idx, src, axis=0):
    return tgt.at[idx].add(src)
def _segment_sum(src, seg, n):
    return jax.ops.segment_sum(src, seg, n)
class _Rng:
    def __init__(self, key):
        self._k = key
    def _next(self):
        self._k, sub = jax.random.split(self._k)
        return sub
    def normal(self, shape):
        return jax.random.normal(self._next(), shape, dtype=jnp.bfloat16)
    def randint(self, lo, hi, shape):
        return jax.random.randint(self._next(), shape, lo, hi, dtype=jnp.int32)
    def uniform(self, shape, lo=0.0, hi=1.0):
        return jax.random.uniform(self._next(), shape, jnp.bfloat16, lo, hi)
    def permutation(self, n):
        return jax.random.permutation(self._next(), n)


kernel_name = 'standalone__fused_io_aware_attn__prompt'

def setup_inputs():
    _rng = _Rng(jax.random.key(int.from_bytes(__import__("os").urandom(4), "little")))
    _w = (lambda a: (lambda t: t.astype(jnp.bfloat16) if jnp.issubdtype(t.dtype, jnp.floating) else t)(jnp.asarray(a)))
    B, H, S = 2, 32, 2048
    Dh = max(1, 1024 // 32)
    return {
        "q": _w((lambda *s: _rng.normal(s) * 0.05)(B, H, S, Dh)),
        "k": _w((lambda *s: _rng.normal(s) * 0.05)(B, H, S, Dh)),
        "v": _w((lambda *s: _rng.normal(s) * 0.05)(B, H, S, Dh)),
    }

def reference(q, k, v):
    scale = q.shape[-1] ** -0.5
    s = jnp.einsum('bhqd,bhkd->bhqk', q, k) * scale
    p = _softmax(s, axis=-1)
    return jnp.einsum('bhqk,bhkd->bhqd', p, v)
```

```python
import jax
import jax.numpy as jnp
from jax import lax
import jax.experimental.pallas as pl
import jax.experimental.pallas.tpu as pltpu

_LOG2E = 1.4426950408889634
_HP = 4
_BK = 256
_LAG = 1
_SBQ = 256
_L_MIN = 2.0 ** -40
_L_MAX = 2.0 ** 80


def _kernel(qt_ref, kt_ref, vt_ref, ot_ref, k_scr):
    _, D, S = qt_ref.shape
    nk = S // _BK
    scale = (D ** -0.5) * _LOG2E

    def fast_head(h):
        ks = k_scr.at[h % 2]
        ks[...] = kt_ref[h].T
        qT = (qt_ref[h].astype(jnp.float32) * scale).astype(jnp.bfloat16)
        l8 = jnp.zeros((8, S), jnp.float32)
        acc = jnp.zeros((D, S), jnp.float32)

        def qk(c):
            return jnp.dot(ks[c * _BK:(c + 1) * _BK, :], qT,
                           preferred_element_type=jnp.float32)

        pend = [qk(c) for c in range(_LAG)]
        for c in range(nk):
            if c + _LAG < nk:
                pend.append(qk(c + _LAG))
            p = jnp.exp2(pend.pop(0))
            l8 = l8 + jnp.sum(p.reshape(_BK // 8, 8, S), axis=0)
            acc = acc + jnp.dot(vt_ref[h, :, c * _BK:(c + 1) * _BK],
                                p.astype(jnp.bfloat16),
                                preferred_element_type=jnp.float32)
        l = jnp.sum(l8, axis=0, keepdims=True)
        o = acc * (1.0 / l)
        ot_ref[h] = o.astype(ot_ref.dtype)
        in_range = (l >= _L_MIN) & (l <= _L_MAX)
        finite = jnp.sum((o * 0.0).reshape(D // 8, 8, S), axis=0) == 0.0
        return jnp.where(in_range & finite, 0, 1).astype(jnp.int32)

    bad = fast_head(0)
    for h in range(1, _HP):
        bad = jnp.maximum(bad, fast_head(h))

    @pl.when(jnp.max(bad) > 0)
    def _true_max_path():
        def head_body(h, carry):
            k_scr[0] = kt_ref[h].T

            def q_body(i, c2):
                q0 = pl.multiple_of(i * _SBQ, _SBQ)
                sT = jnp.dot(k_scr[0], qt_ref[h, :, pl.ds(q0, _SBQ)],
                             preferred_element_type=jnp.float32)
                m = jnp.max(sT, axis=0, keepdims=True)
                p = jnp.exp2((sT - m) * scale)
                l = jnp.sum(p, axis=0, keepdims=True)
                o = jnp.dot(vt_ref[h], p.astype(jnp.bfloat16),
                            preferred_element_type=jnp.float32)
                ot_ref[h, :, pl.ds(q0, _SBQ)] = (o / l).astype(ot_ref.dtype)
                return c2

            return lax.fori_loop(0, S // _SBQ, q_body, carry)

        lax.fori_loop(0, _HP, head_body, 0)


@jax.jit
def pallas_standalone__fused_io_aware_attn__prompt_kernel(
    q: jax.Array,
    k: jax.Array,
    v: jax.Array,
):
    B, H, S, D = q.shape

    def t(x):
        return x.transpose(0, 1, 3, 2).reshape(B * H, D, S)

    spec = pl.BlockSpec((_HP, D, S), lambda g: (g, 0, 0))
    o = pl.pallas_call(
        _kernel,
        grid=(B * H // _HP,),
        in_specs=[spec, spec, spec],
        out_specs=spec,
        out_shape=jax.ShapeDtypeStruct((B * H, D, S), q.dtype),
        scratch_shapes=[pltpu.VMEM((2, S, D), jnp.bfloat16)],
        compiler_params=pltpu.CompilerParams(
            dimension_semantics=("parallel",),
            vmem_limit_bytes=100 * 2 ** 20,
        ),
    )(t(q), t(k), t(v))
    return o.reshape(B, H, D, S).transpose(0, 1, 3, 2)
```

```python
import jax
import jax.numpy as jnp
from jax import lax
import jax.experimental.pallas as pl
import jax.experimental.pallas.tpu as pltpu

_LOG2E = 1.4426950408889634
_HP = 4
_BK = 256
_LAG = 1
_SBQ = 256
_L_MIN = 2.0 ** -40
_L_MAX = 2.0 ** 80
_ACC_MIN = 2.0 ** -90
_ACC_MAX = 2.0 ** 126


def _kernel(qt_ref, kt_ref, vt_ref, ot_ref, k_scr):
    _, D, S = qt_ref.shape
    nk = S // _BK
    scale = (D ** -0.5) * _LOG2E

    def fast_head(h):
        ks = k_scr.at[h % 2]
        ks[...] = kt_ref[h].T
        qT = (qt_ref[h].astype(jnp.float32) * scale).astype(jnp.bfloat16)
        l8 = jnp.zeros((8, S), jnp.float32)
        acc = jnp.zeros((D, S), jnp.float32)

        def qk(c):
            return jnp.dot(ks[c * _BK:(c + 1) * _BK, :], qT,
                           preferred_element_type=jnp.float32)

        pend = [qk(c) for c in range(_LAG)]
        for c in range(nk):
            if c + _LAG < nk:
                pend.append(qk(c + _LAG))
            p = jnp.exp2(pend.pop(0))
            l8 = l8 + jnp.sum(p.reshape(_BK // 8, 8, S), axis=0)
            acc = acc + jnp.dot(vt_ref[h, :, c * _BK:(c + 1) * _BK],
                                p.astype(jnp.bfloat16),
                                preferred_element_type=jnp.float32)
        l = jnp.sum(l8, axis=0, keepdims=True)
        o = acc * (1.0 / l)
        ot_ref[h] = o.astype(ot_ref.dtype)
        a = jnp.abs(acc).reshape(D // 8, 8, S)
        safe = ((l >= _L_MIN) & (l <= _L_MAX)
                & (jnp.min(a, axis=0) >= _ACC_MIN)
                & (jnp.max(a, axis=0) <= _ACC_MAX))
        return jnp.where(safe, 0, 1).astype(jnp.int32)

    bad = fast_head(0)
    for h in range(1, _HP):
        bad = jnp.maximum(bad, fast_head(h))

    @pl.when(jnp.max(bad) > 0)
    def _true_max_path():
        def head_body(h, carry):
            k_scr[0] = kt_ref[h].T

            def q_body(i, c2):
                q0 = pl.multiple_of(i * _SBQ, _SBQ)
                sT = jnp.dot(k_scr[0], qt_ref[h, :, pl.ds(q0, _SBQ)],
                             preferred_element_type=jnp.float32)
                m = jnp.max(sT, axis=0, keepdims=True)
                p = jnp.exp2((sT - m) * scale)
                l = jnp.sum(p, axis=0, keepdims=True)
                o = jnp.dot(vt_ref[h], p.astype(jnp.bfloat16),
                            preferred_element_type=jnp.float32)
                ot_ref[h, :, pl.ds(q0, _SBQ)] = (o / l).astype(ot_ref.dtype)
                return c2

            return lax.fori_loop(0, S // _SBQ, q_body, carry)

        lax.fori_loop(0, _HP, head_body, 0)


@jax.jit
def pallas_standalone__fused_io_aware_attn__prompt_kernel(
    q: jax.Array,
    k: jax.Array,
    v: jax.Array,
):
    B, H, S, D = q.shape

    def t(x):
        return x.transpose(0, 1, 3, 2).reshape(B * H, D, S)

    spec = pl.BlockSpec((_HP, D, S), lambda g: (g, 0, 0))
    o = pl.pallas_call(
        _kernel,
        grid=(B * H // _HP,),
        in_specs=[spec, spec, spec],
        out_specs=spec,
        out_shape=jax.ShapeDtypeStruct((B * H, D, S), q.dtype),
        scratch_shapes=[pltpu.VMEM((2, S, D), jnp.bfloat16)],
        compiler_params=pltpu.CompilerParams(
            dimension_semantics=("parallel",),
            vmem_limit_bytes=100 * 2 ** 20,
        ),
    )(t(q), t(k), t(v))
    return o.reshape(B, H, D, S).transpose(0, 1, 3, 2)
```

```python
import jax
import jax.numpy as jnp
from jax import lax
import jax.experimental.pallas as pl
import jax.experimental.pallas.tpu as pltpu

_LOG2E = 1.4426950408889634
_HP = 4
_BK = 256
_LAG = 1
_SBQ = 256
_L_MIN = 2.0 ** -40
_L_MAX = 2.0 ** 80
_V_MIN = 2.0 ** -40
_ACC_MAX = 2.0 ** 126


def _kernel(qt_ref, kt_ref, vt_ref, ot_ref, k_scr):
    _, D, S = qt_ref.shape
    nk = S // _BK
    scale = (D ** -0.5) * _LOG2E

    def fast_head(h):
        ks = k_scr.at[h % 2]
        ks[...] = kt_ref[h].T
        qT = (qt_ref[h].astype(jnp.float32) * scale).astype(jnp.bfloat16)
        l8 = jnp.zeros((8, S), jnp.float32)
        acc = jnp.zeros((D, S), jnp.float32)

        def qk(c):
            return jnp.dot(ks[c * _BK:(c + 1) * _BK, :], qT,
                           preferred_element_type=jnp.float32)

        pend = [qk(c) for c in range(_LAG)]
        for c in range(nk):
            if c + _LAG < nk:
                pend.append(qk(c + _LAG))
            p = jnp.exp2(pend.pop(0))
            l8 = l8 + jnp.sum(p.reshape(_BK // 8, 8, S), axis=0)
            acc = acc + jnp.dot(vt_ref[h, :, c * _BK:(c + 1) * _BK],
                                p.astype(jnp.bfloat16),
                                preferred_element_type=jnp.float32)
        l = jnp.sum(l8, axis=0, keepdims=True)
        o = acc * (1.0 / l)
        ot_ref[h] = o.astype(ot_ref.dtype)
        amax = jnp.max(jnp.abs(acc).reshape(D // 8, 8, S), axis=0)
        v_abs = jnp.abs(vt_ref[h].astype(jnp.float32))
        v_abs = jnp.where(v_abs == 0.0, 1.0, v_abs)
        vmin = jnp.min(v_abs.reshape(D // 8, 8, S), axis=0)
        safe = ((l >= _L_MIN) & (l <= _L_MAX)
                & (amax <= _ACC_MAX) & (vmin >= _V_MIN))
        return jnp.where(safe, 0, 1).astype(jnp.int32)

    bad = fast_head(0)
    for h in range(1, _HP):
        bad = jnp.maximum(bad, fast_head(h))

    @pl.when(jnp.max(bad) > 0)
    def _true_max_path():
        def head_body(h, carry):
            k_scr[0] = kt_ref[h].T

            def q_body(i, c2):
                q0 = pl.multiple_of(i * _SBQ, _SBQ)
                sT = jnp.dot(k_scr[0], qt_ref[h, :, pl.ds(q0, _SBQ)],
                             preferred_element_type=jnp.float32)
                m = jnp.max(sT, axis=0, keepdims=True)
                p = jnp.exp2((sT - m) * scale)
                l = jnp.sum(p, axis=0, keepdims=True)
                o = jnp.dot(vt_ref[h], p.astype(jnp.bfloat16),
                            preferred_element_type=jnp.float32)
                ot_ref[h, :, pl.ds(q0, _SBQ)] = (o / l).astype(ot_ref.dtype)
                return c2

            return lax.fori_loop(0, S // _SBQ, q_body, carry)

        lax.fori_loop(0, _HP, head_body, 0)


@jax.jit
def pallas_standalone__fused_io_aware_attn__prompt_kernel(
    q: jax.Array,
    k: jax.Array,
    v: jax.Array,
):
    B, H, S, D = q.shape

    def t(x):
        return x.transpose(0, 1, 3, 2).reshape(B * H, D, S)

    spec = pl.BlockSpec((_HP, D, S), lambda g: (g, 0, 0))
    o = pl.pallas_call(
        _kernel,
        grid=(B * H // _HP,),
        in_specs=[spec, spec, spec],
        out_specs=spec,
        out_shape=jax.ShapeDtypeStruct((B * H, D, S), q.dtype),
        scratch_shapes=[pltpu.VMEM((2, S, D), jnp.bfloat16)],
        compiler_params=pltpu.CompilerParams(
            dimension_semantics=("parallel",),
            vmem_limit_bytes=100 * 2 ** 20,
        ),
    )(t(q), t(k), t(v))
    return o.reshape(B, H, D, S).transpose(0, 1, 3, 2)
```
